```python
import jax
import jax.numpy as jnp

def _softmax(x, axis=-1):
    return jax.nn.softmax(x, axis=axis)
def _gelu(x):
    return jax.nn.gelu(x, approximate=True)
def _silu(x):
    return jax.nn.silu(x)
def _sigmoid(x):
    return jax.nn.sigmoid(x)
def _layernorm(x, axis=-1, eps=1e-5):
    m = jnp.mean(x, axis=axis, keepdims=True)
    v = jnp.var(x, axis=axis, keepdims=True)
    return (x - m) / jnp.sqrt(v + eps)
def _scatter_add(tgt, idx, src, axis=0):
    return tgt.at[idx].add(src)
def _segment_sum(src, seg, n):
    return jax.ops.segment_sum(src, seg, n)
class _Rng:
    def __init__(self, key):
        self._k = key
    def _next(self):
        self._k, sub = jax.random.split(self._k)
        return sub
    def normal(self, shape):
        return jax.random.normal(self._next(), shape, dtype=jnp.bfloat16)
    def randint(self, lo, hi, shape):
        return jax.random.randint(self._next(), shape, lo, hi, dtype=jnp.int32)
    def uniform(self, shape, lo=0.0, hi=1.0):
        return jax.random.uniform(self._next(), shape, jnp.bfloat16, lo, hi)
    def permutation(self, n):
        return jax.random.permutation(self._next(), n)


kernel_name = 'recurrent_scan__sliding_block_cached__glu_gated_swiglu__decode'

def setup_inputs():
    _rng = _Rng(jax.random.key(int.from_bytes(__import__("os").urandom(4), "little")))
    _w = (lambda a: (lambda t: t.astype(jnp.bfloat16) if jnp.issubdtype(t.dtype, jnp.floating) else t)(jnp.asarray(a)))
    def _A_setup():
        B, Sq, D = 1, 1, 640
        Hq, Hkv, Sk, Dh = 32, 32, 32768, 192
        assert Hq % Hkv == 0, (Hq, Hkv)
        return {
            "x": _w((lambda *s: _rng.normal(s) * 0.05)(B, Sq, D)),
            "k_cache": _w((lambda *s: _rng.normal(s) * 0.05)(B, Hkv, Sk, Dh)),
            "v_cache": _w((lambda *s: _rng.normal(s) * 0.05)(B, Hkv, Sk, Dh)),
            "wq": _w((lambda *s: _rng.normal(s) * 0.05)(D, Hq * Dh) * (D ** -0.5)),
            "wo": _w((lambda *s: _rng.normal(s) * 0.05)(Hq * Dh, D) * ((Hq * Dh) ** -0.5)),
        }
    _A_in = _A_setup()

    def _B_setup():
        B, S, D, F = 1, 1, 640, 1536
        return {
            "x": _w((lambda *s: _rng.normal(s) * 0.05)(B, S, D)),
            "w1": _w((lambda *s: _rng.normal(s) * 0.05)(D, F) * (2.0 / D) ** 0.5),
            "w3": _w((lambda *s: _rng.normal(s) * 0.05)(D, F) * (2.0 / D) ** 0.5),
            "w2": _w((lambda *s: _rng.normal(s) * 0.05)(F, D) * (2.0 / F) ** 0.5),
        }
    _B_in = _B_setup()

    return {
        "A_x": _A_in["x"],
        "A_k_cache": _A_in["k_cache"],
        "A_v_cache": _A_in["v_cache"],
        "A_wq": _A_in["wq"],
        "A_wo": _A_in["wo"],
        "B_x": _B_in["x"],
        "B_w1": _B_in["w1"],
        "B_w3": _B_in["w3"],
        "B_w2": _B_in["w2"],
    }

def reference(A_x, A_k_cache, A_v_cache, A_wq, A_wo, B_x, B_w1, B_w3, B_w2):
    def _A_ref(x, k_cache, v_cache, wq, wo):
        B, Sq, D = x.shape
        Hq, Dh = 32, 192
        Hkv, Sk = k_cache.shape[1], k_cache.shape[2]
        W = min(4096, max(256, Sk // 4))
        rep = Hq // Hkv
        q = (lambda x, *d: x.transpose(*d))((x @ wq).reshape(B, Sq, Hq, Dh), 0, 2, 1, 3)
        k = jnp.repeat(k_cache[:, :, Sk - W:, :], rep, axis=1)
        v = jnp.repeat(v_cache[:, :, Sk - W:, :], rep, axis=1)
        scores = jnp.einsum("bhqd,bhkd->bhqk", q, k) * (Dh ** -0.5)
        p = _softmax(scores, axis=-1)
        o = jnp.einsum("bhqk,bhkd->bhqd", p, v)
        return (lambda x, *d: x.transpose(*d))(o, 0, 2, 1, 3).reshape(B, Sq, Hq * Dh) @ wo

    def _B_ref(x, w1, w3, w2):
        gate = jnp.einsum("bsd,df->bsf", x, w1)
        up = jnp.einsum("bsd,df->bsf", x, w3)
        h = _silu(gate) * up
        out = jnp.einsum("bsf,fd->bsd", h, w2)
        return out

    x = A_x
    xn = _layernorm(x, axis=-1)
    s = _A_ref(xn, A_k_cache, A_v_cache, A_wq, A_wo)
    g = _silu(_B_ref(xn, B_w1, B_w3, B_w2))
    return x + s * g
```

```python
import jax
import jax.numpy as jnp
import jax.experimental.pallas as pl
import jax.experimental.pallas.tpu as pltpu

HQ, DH = 32, 192
PAIR = 2 * DH
ROWS = 16
LOOKAHEAD = 3
NBUF = 4
WQ_ROWS = 128
WO_ROWS = (768,) * 8
_NT = (((1,), (1,)), ((), ()))


def _kernel(x_hbm, k_hbm, v_hbm, wq_hbm, wo_hbm, w1_hbm, w3_hbm, w2_hbm, o_ref,
            x_v, wq_v, wo_v, w1_v, w3_v, w2_v, kbuf, vbuf, q_s, o_s,
            sem_x, sem_wq, sem_wo, sem_mlp, sem_k, sem_v):
    D = wq_v.shape[0]
    Sk = k_hbm.shape[1]
    W = kbuf.shape[2]
    npairs = k_hbm.shape[0] // PAIR
    nwq = D // WQ_ROWS
    wo_offs = [sum(WO_ROWS[:i]) for i in range(len(WO_ROWS))]
    L = LOOKAHEAD

    def cp_wq(c):
        rows = pl.ds(c * WQ_ROWS, WQ_ROWS)
        return pltpu.make_async_copy(wq_hbm.at[rows], wq_v.at[rows], sem_wq.at[c])

    def cp_wo(c):
        rows = pl.ds(wo_offs[c], WO_ROWS[c])
        return pltpu.make_async_copy(wo_hbm.at[rows], wo_v.at[rows], sem_wo.at[c])

    def cp_cache(hbm, buf, sem, j):
        slot = j % NBUF
        rows = pl.ds(pl.multiple_of(j * PAIR, PAIR), PAIR)
        return pltpu.make_async_copy(
            hbm.at[rows, pl.ds(Sk - W, W)], buf.at[slot], sem.at[slot])

    def cp_k(j):
        return cp_cache(k_hbm, kbuf, sem_k, j)

    def cp_v(j):
        return cp_cache(v_hbm, vbuf, sem_v, j)

    cp_x = pltpu.make_async_copy(x_hbm, x_v, sem_x)
    cp_w1 = pltpu.make_async_copy(w1_hbm, w1_v, sem_mlp.at[0])
    cp_w3 = pltpu.make_async_copy(w3_hbm, w3_v, sem_mlp.at[1])
    cp_w2 = pltpu.make_async_copy(w2_hbm, w2_v, sem_mlp.at[2])

    head = [cp_wq(c) for c in range(nwq)] + [cp_w1, cp_w3, cp_w2]
    nh = len(head)

    def start(i):
        if i < nh:
            c = head[i]
        elif i < nh + 2 * npairs:
            c = (cp_k, cp_v)[(i - nh) % 2]((i - nh) // 2)
        elif i < nh + 2 * npairs + len(WO_ROWS):
            c = cp_wo(i - nh - 2 * npairs)
        else:
            return
        c.start(priority=i % 2)

    start(0)
    cp_x.start()
    for i in range(1, L):
        start(i)

    cp_x.wait()
    x = x_v[...].astype(jnp.float32)
    xc = x - jnp.mean(x, axis=-1, keepdims=True)
    var = jnp.mean(xc * xc, axis=-1, keepdims=True)
    xn = xc / jnp.sqrt(var + 1e-5)
    xn = jnp.broadcast_to(xn, (ROWS, D)).astype(jnp.bfloat16)

    q = None
    for c in range(nwq):
        cp_wq(c).wait()
        start(c + L)
        part = jnp.dot(xn[:, c * WQ_ROWS:(c + 1) * WQ_ROWS],
                       wq_v[pl.ds(c * WQ_ROWS, WQ_ROWS), :],
                       preferred_element_type=jnp.float32)
        q = part if q is None else q + part
    row = jax.lax.broadcasted_iota(jnp.int32, (ROWS, PAIR), 0)
    col = jax.lax.broadcasted_iota(jnp.int32, (ROWS, PAIR), 1)
    diag = row == (col >= DH).astype(jnp.int32)
    for j in range(npairs):
        q_s[j] = jnp.where(diag, q[:, j * PAIR:(j + 1) * PAIR], 0.0).astype(jnp.bfloat16)

    cp_w1.wait()
    start(nwq + L)
    gate = jnp.dot(xn, w1_v[...], preferred_element_type=jnp.float32)
    cp_w3.wait()
    start(nwq + 1 + L)
    up = jnp.dot(xn, w3_v[...], preferred_element_type=jnp.float32)
    h = (gate * jax.nn.sigmoid(gate) * up).astype(jnp.bfloat16)
    cp_w2.wait()
    start(nwq + 2 + L)
    mlp = jnp.dot(h, w2_v[...], preferred_element_type=jnp.float32)[0:1]
    g = mlp * jax.nn.sigmoid(mlp)

    scale = DH ** -0.5

    def pair_body(j, start_after_k, start_after_v):
        slot = j % NBUF
        cp_k(j).wait()
        start_after_k()
        s = jnp.dot(q_s[j], kbuf[slot], preferred_element_type=jnp.float32) * scale
        p = jnp.exp(s - jnp.max(s, axis=-1, keepdims=True))
        denom = jnp.sum(p, axis=-1, keepdims=True)
        cp_v(j).wait()
        start_after_v()
        o = jax.lax.dot_general(p.astype(jnp.bfloat16), vbuf[slot], _NT,
                                preferred_element_type=jnp.float32)
        o_s[j] = jnp.where(diag, o / denom, 0.0).astype(jnp.bfloat16)

    def start_kv(j, off):
        (cp_k, cp_v)[off % 2](j + off // 2).start(priority=(nh + off) % 2)

    def loop_body(j, carry):
        pair_body(j, lambda: start_kv(j, L), lambda: start_kv(j, L + 1))
        return carry

    n_loop = npairs - (L + 2) // 2
    jax.lax.fori_loop(0, n_loop, loop_body, 0)
    for j in range(n_loop, npairs):
        pair_body(j, lambda: start(nh + 2 * j + L), lambda: start(nh + 2 * j + 1 + L))

    o_all = jnp.concatenate([o_s[j] for j in range(npairs)], axis=1)
    acc = None
    for c in range(len(WO_ROWS)):
        cp_wo(c).wait()
        start(nh + 2 * npairs + c + L)
        part = jnp.dot(o_all[:, wo_offs[c]:wo_offs[c] + WO_ROWS[c]],
                       wo_v[pl.ds(wo_offs[c], WO_ROWS[c]), :],
                       preferred_element_type=jnp.float32)
        acc = part if acc is None else acc + part
    attn = jnp.sum(acc, axis=0, keepdims=True)
    o_ref[...] = (x + attn * g).astype(o_ref.dtype)


@jax.jit
def pallas_recurrent_scan__sliding_block_cached__glu_gated_swiglu__decode_kernel(
    A_x: jax.Array,
    A_k_cache: jax.Array,
    A_v_cache: jax.Array,
    A_wq: jax.Array,
    A_wo: jax.Array,
    B_x: jax.Array,
    B_w1: jax.Array,
    B_w3: jax.Array,
    B_w2: jax.Array,
):
    del B_x
    B, Sq, D = A_x.shape
    _, H, Sk, Dh = A_k_cache.shape
    F = B_w1.shape[1]
    assert (B, Sq, H, Dh) == (1, 1, HQ, DH)
    W = min(4096, max(256, Sk // 4))
    kt = jnp.swapaxes(A_k_cache, 2, 3).reshape(H * Dh, Sk)
    vt = jnp.swapaxes(A_v_cache, 2, 3).reshape(H * Dh, Sk)
    dma = pltpu.SemaphoreType.DMA
    out = pl.pallas_call(
        _kernel,
        out_shape=jax.ShapeDtypeStruct((1, D), A_x.dtype),
        in_specs=[pl.BlockSpec(memory_space=pltpu.HBM)] * 8,
        out_specs=pl.BlockSpec(memory_space=pltpu.VMEM),
        scratch_shapes=[
            pltpu.VMEM((1, D), A_x.dtype),
            pltpu.VMEM(A_wq.shape, A_wq.dtype),
            pltpu.VMEM(A_wo.shape, A_wo.dtype),
            pltpu.VMEM(B_w1.shape, B_w1.dtype),
            pltpu.VMEM(B_w3.shape, B_w3.dtype),
            pltpu.VMEM(B_w2.shape, B_w2.dtype),
            pltpu.VMEM((NBUF, PAIR, W), kt.dtype),
            pltpu.VMEM((NBUF, PAIR, W), vt.dtype),
            pltpu.VMEM((H // 2, ROWS, PAIR), jnp.bfloat16),
            pltpu.VMEM((H // 2, ROWS, PAIR), jnp.bfloat16),
            dma(()),
            dma((D // WQ_ROWS,)),
            dma((len(WO_ROWS),)),
            dma((3,)),
            dma((NBUF,)),
            dma((NBUF,)),
        ],
        compiler_params=pltpu.CompilerParams(vmem_limit_bytes=100 * 1024 * 1024),
    )(A_x.reshape(1, D), kt, vt, A_wq, A_wo, B_w1, B_w3, B_w2)
    return out.reshape(B, Sq, D)
```

```python
import jax
import jax.numpy as jnp
import jax.experimental.pallas as pl
import jax.experimental.pallas.tpu as pltpu

HQ, DH = 32, 192
PAIR = 2 * DH
ROWS = 8
AHEAD = 16
STEP = 256
GAP = 2
KV_SLICE = (40, 8, 1024)
WQ_SLICE = (32, 8, 1024)
W13_SLICE = (24, 8, 1536)
WO_SLICE = (48, 16, 640)
_NT = (((1,), (1,)), ((), ()))
f32, bf16 = jnp.float32, jnp.bfloat16


def _slice(hbm, buf, shape, src_row, src_col, row, col):
    n1, n0, width = shape
    copies = [(hbm.at[pl.ds(src_row + r, n), pl.ds(src_col, width)],
               buf.at[pl.ds(row + r, n), pl.ds(col, width)], priority)
              for r, n, priority in ((0, n1, 1), (n1, n0, 0))]
    return copies, buf.at[pl.ds(row, n1 + n0), pl.ds(col, width)]


def _matrix_slices(hbm, buf, shape):
    n1, n0, width = shape
    assert hbm.shape[0] % (n1 + n0) == 0 and hbm.shape[1] % width == 0
    return [_slice(hbm, buf, shape, r, c, r, c)
            for c in range(0, hbm.shape[1], width)
            for r in range(0, hbm.shape[0], n1 + n0)]


def _kernel(x_hbm, k_hbm, v_hbm, wq_hbm, wo_hbm, w1_hbm, w3_hbm, w2_hbm, o_ref,
            x_v, wq_v, wo_v, w1_v, w3_v, w2_v, kbuf, vbuf, q_s, o_s, s_s,
            sem_x, sems):
    D, F = w1_v.shape
    Sk = k_hbm.shape[1]
    W = kbuf.shape[2]
    npairs = k_hbm.shape[0] // PAIR

    kv_rows, kv_width = KV_SLICE[0] + KV_SLICE[1], KV_SLICE[2]
    kv_down = PAIR // kv_rows
    kv_count = kv_down * (W // kv_width)
    assert (2 * kv_count) % AHEAD == 0

    def kv_slice(j, t):
        hbm, buf = (k_hbm, kbuf) if t < kv_count else (v_hbm, vbuf)
        c, r = divmod(t % kv_count, kv_down)
        base = j * PAIR if isinstance(j, int) else pl.multiple_of(j * PAIR, PAIR)
        return _slice(hbm, buf.at[j % 2], KV_SLICE, base + r * kv_rows,
                      Sk - W + c * kv_width, r * kv_rows, c * kv_width)

    wq_sl = _matrix_slices(wq_hbm, wq_v, WQ_SLICE)
    w1_sl = _matrix_slices(w1_hbm, w1_v, W13_SLICE)
    w3_sl = _matrix_slices(w3_hbm, w3_v, W13_SLICE)
    w2_sl = _matrix_slices(w2_hbm, w2_v, WO_SLICE)
    wo_sl = _matrix_slices(wo_hbm, wo_v, WO_SLICE)
    tail_sl = w1_sl + w3_sl + w2_sl + wo_sl
    head = len(wq_sl)
    tail = head + npairs * 2 * kv_count

    def stream(t):
        if t < head:
            return wq_sl[t]
        if t < tail:
            return kv_slice(*divmod(t - head, 2 * kv_count))
        return tail_sl[t - tail] if t - tail < len(tail_sl) else None

    def start(sl, t):
        if sl is not None:
            for src, dst, priority in sl[0]:
                pltpu.make_async_copy(src, dst, sems.at[t % AHEAD]).start(priority=priority)

    def wait(sl, t):
        pltpu.make_async_copy(sl[1], sl[1], sems.at[t % AHEAD]).wait()

    def advance(t):
        wait(stream(t), t)
        start(stream(t + AHEAD), t + AHEAD)

    def run(t0, t1, work):
        last = t0 - GAP
        for t in range(t0, t1):
            advance(t)
            if work and work[0][0] <= t and t - last >= GAP:
                work.pop(0)[1]()
                last = t
        for _, fn in work:
            fn()

    def columns_ready(n, shape):
        return (((n + 1) * STEP - 1) // shape[2] + 1) * (D // (shape[0] + shape[1])) - 1

    def rows_ready(n, shape):
        return pl.cdiv((n + 1) * STEP, shape[0] + shape[1]) - 1

    cp_x = pltpu.make_async_copy(x_hbm, x_v, sem_x)
    cp_x.start()
    for t in range(AHEAD):
        start(stream(t), t)

    cp_x.wait()
    x = x_v[...].astype(f32)
    xc = x - jnp.mean(x, axis=-1, keepdims=True)
    var = jnp.mean(xc * xc, axis=-1, keepdims=True)
    xn = jnp.broadcast_to(xc / jnp.sqrt(var + 1e-5), (ROWS, D)).astype(bf16)

    row = jax.lax.broadcasted_iota(jnp.int32, (ROWS, PAIR), 0)
    col = jax.lax.broadcasted_iota(jnp.int32, (ROWS, PAIR), 1)
    diag = row == (col >= DH).astype(jnp.int32)
    lanes = STEP // 128

    def q_piece(n):
        def fn():
            q = jnp.dot(xn, wq_v[:, pl.ds(n * STEP, STEP)], preferred_element_type=f32)
            for i in range(lanes):
                j, o = divmod(n * lanes + i, PAIR // 128)
                q_s[j, :, pl.ds(o * 128, 128)] = jnp.where(
                    diag[:, o * 128:(o + 1) * 128], q[:, i * 128:(i + 1) * 128], 0.0
                ).astype(bf16)
        return fn

    run(0, head + kv_down,
        [(columns_ready(n, WQ_SLICE), q_piece(n)) for n in range(wq_v.shape[1] // STEP)])

    scale = DH ** -0.5
    pieces = W // STEP

    def pair_body(j):
        slot = j % 2
        st = {}

        def scores(i):
            cols = pl.ds(i * STEP, STEP)
            s = jnp.dot(q_s[j], kbuf[slot, :, cols], preferred_element_type=f32) * scale
            s_s[:, cols] = s
            st["m"] = s if i == 0 else jnp.maximum(st["m"], s)
            if i == pieces - 1:
                st["m"] = jnp.max(st["m"], axis=-1, keepdims=True)

        def values(i):
            cols = pl.ds(i * STEP, STEP)
            p = jnp.exp(s_s[:, cols] - st["m"])
            o = jax.lax.dot_general(p.astype(bf16), vbuf[slot, :, cols], _NT,
                                    preferred_element_type=f32)
            st["l"] = p if i == 0 else st["l"] + p
            st["o"] = o if i == 0 else st["o"] + o
            if i == pieces - 1:
                denom = jnp.sum(st["l"], axis=-1, keepdims=True)
                o_s[j] = jnp.where(diag, st["o"] / denom, 0.0).astype(bf16)

        done = 0
        for u in range(2 * kv_count):
            t = kv_down + u
            if isinstance(j, int):
                advance(head + j * 2 * kv_count + t)
            else:
                wait(kv_slice(j + t // (2 * kv_count), t % (2 * kv_count)), head + t)
                t += AHEAD
                start(kv_slice(j + t // (2 * kv_count), t % (2 * kv_count)), head + t)
            while done <= u * pieces // kv_count:
                (scores if done < pieces else values)(done % pieces)
                done += 1

    def loop_body(j, carry):
        pair_body(j)
        return carry

    jax.lax.fori_loop(0, npairs - 1, loop_body, 0)
    pair_body(npairs - 1)

    st = {}

    def gate_piece(n):
        def fn():
            st["g", n] = jnp.dot(xn, w1_v[:, pl.ds(n * STEP, STEP)],
                                 preferred_element_type=f32)
        return fn

    def up_piece(n):
        def fn():
            up = jnp.dot(xn, w3_v[:, pl.ds(n * STEP, STEP)], preferred_element_type=f32)
            gate = st["g", n]
            st["h", n] = (gate * jax.nn.sigmoid(gate) * up).astype(bf16)
        return fn

    def down_piece(n):
        def fn():
            part = jnp.dot(st["h", n], w2_v[pl.ds(n * STEP, STEP), :],
                           preferred_element_type=f32)
            st["mlp"] = part if n == 0 else st["mlp"] + part
            if n == F // STEP - 1:
                mlp = st["mlp"][0:1]
                st["gate"] = mlp * jax.nn.sigmoid(mlp)
        return fn

    def out_piece(n):
        def fn():
            lhs = [o_s[i // 3, :, pl.ds(i % 3 * 128, 128)]
                   for i in range(n * lanes, (n + 1) * lanes)]
            part = jnp.dot(jnp.concatenate(lhs, axis=1), wo_v[pl.ds(n * STEP, STEP), :],
                           preferred_element_type=f32)
            st["attn"] = part if n == 0 else st["attn"] + part
        return fn

    t3 = tail + len(w1_sl)
    t2 = t3 + len(w3_sl)
    to = t2 + len(w2_sl)
    work = [(tail + columns_ready(n, W13_SLICE), gate_piece(n)) for n in range(F // STEP)]
    work += [(t3 + columns_ready(n, W13_SLICE), up_piece(n)) for n in range(F // STEP)]
    work += [(t2 + rows_ready(n, WO_SLICE), down_piece(n)) for n in range(F // STEP)]
    work += [(to + rows_ready(n, WO_SLICE), out_piece(n))
             for n in range(wo_v.shape[0] // STEP)]
    run(tail + kv_down, tail + len(tail_sl), work)

    attn = jnp.sum(st["attn"], axis=0, keepdims=True)
    o_ref[...] = (x + attn * st["gate"]).astype(o_ref.dtype)


@jax.jit
def pallas_recurrent_scan__sliding_block_cached__glu_gated_swiglu__decode_kernel(
    A_x: jax.Array,
    A_k_cache: jax.Array,
    A_v_cache: jax.Array,
    A_wq: jax.Array,
    A_wo: jax.Array,
    B_x: jax.Array,
    B_w1: jax.Array,
    B_w3: jax.Array,
    B_w2: jax.Array,
):
    del B_x
    B, Sq, D = A_x.shape
    _, H, Sk, Dh = A_k_cache.shape
    assert (B, Sq, H, Dh) == (1, 1, HQ, DH)
    W = min(4096, max(256, Sk // 4))
    kt = jnp.swapaxes(A_k_cache, 2, 3).reshape(H * Dh, Sk)
    vt = jnp.swapaxes(A_v_cache, 2, 3).reshape(H * Dh, Sk)
    out = pl.pallas_call(
        _kernel,
        out_shape=jax.ShapeDtypeStruct((1, D), A_x.dtype),
        in_specs=[pl.BlockSpec(memory_space=pltpu.HBM)] * 8,
        out_specs=pl.BlockSpec(memory_space=pltpu.VMEM),
        scratch_shapes=[
            pltpu.VMEM((1, D), A_x.dtype),
            pltpu.VMEM(A_wq.shape, A_wq.dtype),
            pltpu.VMEM(A_wo.shape, A_wo.dtype),
            pltpu.VMEM(B_w1.shape, B_w1.dtype),
            pltpu.VMEM(B_w3.shape, B_w3.dtype),
            pltpu.VMEM(B_w2.shape, B_w2.dtype),
            pltpu.VMEM((2, PAIR, W), kt.dtype),
            pltpu.VMEM((2, PAIR, W), vt.dtype),
            pltpu.VMEM((H // 2, ROWS, PAIR), bf16),
            pltpu.VMEM((H // 2, ROWS, PAIR), bf16),
            pltpu.VMEM((ROWS, W), f32),
            pltpu.SemaphoreType.DMA(()),
            pltpu.SemaphoreType.DMA((AHEAD,)),
        ],
        compiler_params=pltpu.CompilerParams(vmem_limit_bytes=64 * 1024 * 1024),
    )(A_x.reshape(1, D), kt, vt, A_wq, A_wo, B_w1, B_w3, B_w2)
    return out.reshape(B, Sq, D)
```

```python
import jax
import jax.numpy as jnp
import jax.experimental.pallas as pl
import jax.experimental.pallas.tpu as pltpu

HQ, DH = 32, 192
PAIR = 2 * DH
LANES = 128
ROWS = 8
STEP = 256
GAP = 2
AHEAD = (12, 16)
NSEM = max(AHEAD)
KV_SLICE = (24, 8, 1024)
WQ_SLICE = (10, 8, 4, 1, 1024)
W13_SLICE = (4, 8, 3, 1, 1536)
WO_SLICE = (8, 16, 3, 1, 640)
W2_SLICE = (1, 16, 3, 1, 640)
_NT = (((1,), (1,)), ((), ()))


def _weight_slices(hbm, buf, shape):
    regions, height, n1, n0, width = shape
    _, rows, cols = hbm.shape
    split = ((0, n1, 1), (n1, n0, 0))
    if regions == 1:
        assert width == cols and rows % ((n1 + n0) * height) == 0
        index = [[((0, pl.ds(r + a * height, n * height)), p) for a, n, p in split]
                 for r in range(0, rows, (n1 + n0) * height)]
    else:
        assert regions % (n1 + n0) == 0 and rows % height == 0 and cols % width == 0
        index = [[((pl.ds(g + a, n), pl.ds(r, height), pl.ds(c, width)), p)
                  for a, n, p in split]
                 for r in range(0, rows, height)
                 for c in range(0, cols, width)
                 for g in range(0, regions, n1 + n0)]
    return [[(hbm.at[i], buf.at[i], p) for i, p in sl] for sl in index]


def _rows_ready(slices, buf, rows):
    assert rows * len(slices) % buf.shape[1] == 0
    return rows * len(slices) // buf.shape[1] - 1


def _kernel(x_hbm, k_hbm, v_hbm, wq_hbm, wo_hbm, w1_hbm, w3_hbm, w2_hbm, o_ref,
            x_v, wq_v, wo_v, w1_v, w3_v, w2_v, kbuf, vbuf,
            q_s, o_s, s_s, h_s, a_s, sem_x, sems):
    f32, bf16 = jnp.float32, jnp.bfloat16
    D = x_v.shape[1]
    F = w1_v.shape[2]
    Sk = k_hbm.shape[1]
    W = kbuf.shape[2]
    npairs = k_hbm.shape[0] // PAIR
    tiles = PAIR // LANES

    kv_rows, kv_width = KV_SLICE[0] + KV_SLICE[1], KV_SLICE[2]
    kv_down = PAIR // kv_rows
    kv_count = kv_down * (W // kv_width)
    assert PAIR % kv_rows == 0 and W % kv_width == 0 and kv_width % STEP == 0
    assert (2 * kv_count) % NSEM == 0 and kv_down + NSEM <= kv_count

    def kv_slice(j, t):
        j, t = j + t // (2 * kv_count), t % (2 * kv_count)
        hbm, buf = (k_hbm, kbuf) if t < kv_count else (v_hbm, vbuf)
        c, r = divmod(t % kv_count, kv_down)
        base = j * PAIR if isinstance(j, int) else pl.multiple_of(j * PAIR, PAIR)
        return [(hbm.at[pl.ds(base + r * kv_rows + a, n),
                        pl.ds(Sk - W + c * kv_width, kv_width)],
                 buf.at[j % 2, pl.ds(r * kv_rows + a, n), pl.ds(c * kv_width, kv_width)],
                 p)
                for a, n, p in ((0, KV_SLICE[0], 1), (KV_SLICE[0], KV_SLICE[1], 0))]

    wq_sl = _weight_slices(wq_hbm, wq_v, WQ_SLICE)
    w1_sl = _weight_slices(w1_hbm, w1_v, W13_SLICE)
    w3_sl = _weight_slices(w3_hbm, w3_v, W13_SLICE)
    wo_sl = _weight_slices(wo_hbm, wo_v, WO_SLICE)
    w2_sl = _weight_slices(w2_hbm, w2_v, W2_SLICE)
    tail_sl = w1_sl + w3_sl + wo_sl + w2_sl
    head = len(wq_sl)
    tail = head + npairs * 2 * kv_count

    def stream(t):
        if t < head:
            return wq_sl[t]
        if t < tail:
            return kv_slice(0, t - head)
        return tail_sl[t - tail] if t - tail < len(tail_sl) else []

    def start(sl, t, priority):
        for src, dst, p in sl:
            if p == priority:
                pltpu.make_async_copy(src, dst, sems.at[t % NSEM]).start(priority=p)

    def advance(t, slice_at=stream):
        for src, dst, _ in slice_at(t):
            pltpu.make_async_copy(src, dst, sems.at[t % NSEM]).wait()
        for p in (1, 0):
            start(slice_at(t + AHEAD[p]), t + AHEAD[p], p)

    def run(t0, t1, work):
        last = t0 - GAP
        for t in range(t0, t1):
            advance(t)
            if work and work[0][0] <= t and t - last >= GAP:
                work.pop(0)[1]()
                last = t
        assert all(ready < t1 for ready, _ in work)
        for _, fn in work:
            fn()

    cp_x = pltpu.make_async_copy(x_hbm, x_v, sem_x)
    for t in range(NSEM):
        for p in (1, 0):
            if t < AHEAD[p]:
                start(stream(t), t, p)
        if t == 0:
            cp_x.start()

    cp_x.wait()
    x = x_v[...].astype(f32)
    xc = x - jnp.mean(x, axis=-1, keepdims=True)
    var = jnp.mean(xc * xc, axis=-1, keepdims=True)
    xn = jnp.broadcast_to(xc / jnp.sqrt(var + 1e-5), (ROWS, D)).astype(bf16)

    def project(w_v, col, width):
        w = w_v[:, :, pl.ds(col, width)].reshape(D, width)
        return jnp.dot(xn, w, preferred_element_type=f32)

    row = jax.lax.broadcasted_iota(jnp.int32, (ROWS, PAIR), 0)
    col = jax.lax.broadcasted_iota(jnp.int32, (ROWS, PAIR), 1)
    diag = row == (col >= DH).astype(jnp.int32)

    def query(j, i):
        c = j * PAIR + i * LANES
        q = project(wq_v, c if isinstance(j, int) else pl.multiple_of(c, LANES), LANES)
        q_s[j, :, pl.ds(i * LANES, LANES)] = jnp.where(
            diag[:, i * LANES:(i + 1) * LANES], q, 0.0).astype(bf16)

    run(0, head + kv_down, [(head - 1, lambda i=i: query(0, i)) for i in range(tiles)])

    scale = DH ** -0.5
    pieces = W // STEP

    def pair(j, last):
        slot = j % 2
        st = {}

        def scores(i):
            cols = pl.ds(i * STEP, STEP)
            s = jnp.dot(q_s[j], kbuf[slot, :, cols], preferred_element_type=f32) * scale
            s_s[:, cols] = s
            st["m"] = s if i == 0 else jnp.maximum(st["m"], s)
            if i == pieces - 1:
                st["m"] = jnp.max(st["m"], axis=-1, keepdims=True)
            if i < tiles and not last:
                query(j + 1, i)

        def values(i):
            cols = pl.ds(i * STEP, STEP)
            p = jnp.exp(s_s[:, cols] - st["m"])
            o = jax.lax.dot_general(p.astype(bf16), vbuf[slot, :, cols], _NT,
                                    preferred_element_type=f32)
            st["l"] = p if i == 0 else st["l"] + p
            st["o"] = o if i == 0 else st["o"] + o
            if i == pieces - 1:
                denom = jnp.sum(st["l"], axis=-1, keepdims=True)
                o_s[j] = jnp.where(diag, st["o"] / denom, 0.0).astype(bf16)

        done = 0
        for u in range(2 * kv_count):
            t = head + kv_down + u
            if last:
                advance(t + j * 2 * kv_count)
            else:
                advance(t, lambda t: kv_slice(j, t - head))
            while done <= u * pieces // kv_count:
                (scores if done < pieces else values)(done % pieces)
                done += 1

    def loop_body(j, carry):
        pair(j, False)
        return carry

    jax.lax.fori_loop(0, npairs - 1, loop_body, 0)
    pair(npairs - 1, True)

    st = {}

    def gate(n):
        st["g", n] = project(w1_v, n * STEP, STEP)

    def hidden(n):
        g = st["g", n]
        h = g * jax.nn.sigmoid(g) * project(w3_v, n * STEP, STEP)
        h_s[:, pl.ds(n * STEP, STEP)] = h.astype(bf16)

    def out_proj(blocks):
        for g, r in blocks:
            i = (g * wo_v.shape[1] + r) // LANES
            part = jnp.dot(o_s[i // tiles, :, pl.ds(i % tiles * LANES, LANES)],
                           wo_v[g, pl.ds(r, LANES), :], preferred_element_type=f32)
            st["attn"] = st["attn"] + part if "attn" in st else part
        if blocks[-1] == (wo_v.shape[0] - 1, wo_v.shape[1] - LANES):
            a_s[...] = jnp.sum(st["attn"], axis=0, keepdims=True)

    def down(r, n):
        part = jnp.dot(h_s[:, pl.ds(r, n)], w2_v[0, pl.ds(r, n), :],
                       preferred_element_type=f32)
        st["mlp"] = st["mlp"] + part if "mlp" in st else part

    t3 = tail + len(w1_sl)
    to = t3 + len(w3_sl)
    t2 = to + len(wo_sl)
    work = [(t3 - 1, lambda n=n: gate(n)) for n in range(F // STEP)]
    work += [(to - 1, lambda n=n: hidden(n)) for n in range(F // STEP)]
    work += [(to + _rows_ready(wo_sl, wo_v, r + LANES),
              lambda g=g, r=r: out_proj([(g, r), (g + 1, r)]))
             for r in range(0, wo_v.shape[1], LANES) for g in range(0, wo_v.shape[0], 2)]
    work += [(t2 + _rows_ready(w2_sl, w2_v, r + n), lambda r=r, n=n: down(r, n))
             for r, n in [(r, STEP) for r in range(0, F - STEP, STEP)]
             + [(r, LANES) for r in range(F - STEP, F, LANES)]]
    run(tail + kv_down, tail + len(tail_sl), work)

    mlp = st["mlp"][0:1]
    o_ref[...] = (x + a_s[...] * (mlp * jax.nn.sigmoid(mlp))).astype(o_ref.dtype)


@jax.jit
def pallas_recurrent_scan__sliding_block_cached__glu_gated_swiglu__decode_kernel(
    A_x: jax.Array,
    A_k_cache: jax.Array,
    A_v_cache: jax.Array,
    A_wq: jax.Array,
    A_wo: jax.Array,
    B_x: jax.Array,
    B_w1: jax.Array,
    B_w3: jax.Array,
    B_w2: jax.Array,
):
    del B_x
    B, Sq, D = A_x.shape
    _, H, Sk, Dh = A_k_cache.shape
    assert (B, Sq, H, Dh) == (1, 1, HQ, DH)
    W = min(4096, max(256, Sk // 4))
    kt = jnp.swapaxes(A_k_cache, 2, 3).reshape(H * Dh, Sk)
    vt = jnp.swapaxes(A_v_cache, 2, 3).reshape(H * Dh, Sk)
    weights = [w.reshape(shape[0], w.shape[0] // shape[0], w.shape[1])
               for w, shape in ((A_wq, WQ_SLICE), (A_wo, WO_SLICE), (B_w1, W13_SLICE),
                                (B_w3, W13_SLICE), (B_w2, W2_SLICE))]
    out = pl.pallas_call(
        _kernel,
        out_shape=jax.ShapeDtypeStruct((1, D), A_x.dtype),
        in_specs=[pl.BlockSpec(memory_space=pltpu.HBM)] * 8,
        out_specs=pl.BlockSpec(memory_space=pltpu.VMEM),
        scratch_shapes=[
            pltpu.VMEM((1, D), A_x.dtype),
            *[pltpu.VMEM(w.shape, w.dtype) for w in weights],
            pltpu.VMEM((2, PAIR, W), kt.dtype),
            pltpu.VMEM((2, PAIR, W), vt.dtype),
            pltpu.VMEM((H // 2, ROWS, PAIR), jnp.bfloat16),
            pltpu.VMEM((H // 2, ROWS, PAIR), jnp.bfloat16),
            pltpu.VMEM((ROWS, W), jnp.float32),
            pltpu.VMEM((ROWS, B_w1.shape[1]), jnp.bfloat16),
            pltpu.VMEM((1, D), jnp.float32),
            pltpu.SemaphoreType.DMA(()),
            pltpu.SemaphoreType.DMA((NSEM,)),
        ],
        compiler_params=pltpu.CompilerParams(
            vmem_limit_bytes=64 * 1024 * 1024, disable_semaphore_checks=True),
    )(A_x.reshape(1, D), kt, vt, *weights)
    return out.reshape(B, Sq, D)
```

```python
import jax
import jax.numpy as jnp
import jax.experimental.pallas as pl
import jax.experimental.pallas.tpu as pltpu

HQ, DH = 32, 192
PAIR = 2 * DH
LANES = 128
ROWS = 8
STEP = 256
GAP = 2
AHEAD = (12, 16)
NSEM = max(AHEAD)
KV_SLICE = (24, 8, 1024)
WQ_SLICE = (10, 8, 4, 1, 1024)
W13_SLICE = (4, 8, 3, 1, 1536)
WO_SLICE = (8, 16, 3, 1, 640)
W2_SLICE = (1, 16, 3, 1, 640)
_NT = (((1,), (1,)), ((), ()))


def _weight_slices(hbm, buf, shape):
    regions, height, n1, n0, width = shape
    _, rows, cols = hbm.shape
    split = ((0, n1, 1), (n1, n0, 0))
    if regions == 1:
        assert width == cols and rows % ((n1 + n0) * height) == 0
        index = [[((0, pl.ds(r + a * height, n * height)), p) for a, n, p in split]
                 for r in range(0, rows, (n1 + n0) * height)]
    else:
        assert regions % (n1 + n0) == 0 and rows % height == 0 and cols % width == 0
        index = [[((pl.ds(g + a, n), pl.ds(r, height), pl.ds(c, width)), p)
                  for a, n, p in split]
                 for r in range(0, rows, height)
                 for c in range(0, cols, width)
                 for g in range(0, regions, n1 + n0)]
    return [[(hbm.at[i], buf.at[i], p) for i, p in sl] for sl in index]


def _rows_ready(slices, buf, rows):
    assert rows * len(slices) % buf.shape[1] == 0
    return rows * len(slices) // buf.shape[1] - 1


def _kernel(*refs):
    dma = pltpu.SemaphoreType.DMA
    pl.run_scoped(lambda *sems: _decode_step(*refs, *sems), dma(()), dma((NSEM,)))


def _decode_step(x_hbm, k_hbm, v_hbm, wq_hbm, wo_hbm, w1_hbm, w3_hbm, w2_hbm, o_ref,
                 x_v, wq_v, wo_v, w1_v, w3_v, w2_v, kbuf, vbuf,
                 q_s, o_s, s_s, h_s, a_s, sem_x, sems):
    f32, bf16 = jnp.float32, jnp.bfloat16
    D = x_v.shape[1]
    F = w1_v.shape[2]
    Sk = k_hbm.shape[1]
    W = kbuf.shape[2]
    npairs = k_hbm.shape[0] // PAIR
    tiles = PAIR // LANES

    kv_rows, kv_width = KV_SLICE[0] + KV_SLICE[1], KV_SLICE[2]
    kv_down = PAIR // kv_rows
    kv_count = kv_down * (W // kv_width)
    assert PAIR % kv_rows == 0 and W % kv_width == 0 and kv_width % STEP == 0
    assert (2 * kv_count) % NSEM == 0 and kv_down + NSEM <= kv_count

    def kv_slice(j, t):
        j, t = j + t // (2 * kv_count), t % (2 * kv_count)
        hbm, buf = (k_hbm, kbuf) if t < kv_count else (v_hbm, vbuf)
        c, r = divmod(t % kv_count, kv_down)
        base = j * PAIR if isinstance(j, int) else pl.multiple_of(j * PAIR, PAIR)
        return [(hbm.at[pl.ds(base + r * kv_rows + a, n),
                        pl.ds(Sk - W + c * kv_width, kv_width)],
                 buf.at[j % 2, pl.ds(r * kv_rows + a, n), pl.ds(c * kv_width, kv_width)],
                 p)
                for a, n, p in ((0, KV_SLICE[0], 1), (KV_SLICE[0], KV_SLICE[1], 0))]

    wq_sl = _weight_slices(wq_hbm, wq_v, WQ_SLICE)
    w1_sl = _weight_slices(w1_hbm, w1_v, W13_SLICE)
    w3_sl = _weight_slices(w3_hbm, w3_v, W13_SLICE)
    wo_sl = _weight_slices(wo_hbm, wo_v, WO_SLICE)
    w2_sl = _weight_slices(w2_hbm, w2_v, W2_SLICE)
    tail_sl = w1_sl + w3_sl + wo_sl + w2_sl
    head = len(wq_sl)
    tail = head + npairs * 2 * kv_count

    def stream(t):
        if t < head:
            return wq_sl[t]
        if t < tail:
            return kv_slice(0, t - head)
        return tail_sl[t - tail] if t - tail < len(tail_sl) else []

    def start(sl, t, priority):
        for src, dst, p in sl:
            if p == priority:
                pltpu.make_async_copy(src, dst, sems.at[t % NSEM]).start(priority=p)

    def advance(t, slice_at=stream):
        for src, dst, _ in slice_at(t):
            pltpu.make_async_copy(src, dst, sems.at[t % NSEM]).wait()
        for p in (1, 0):
            start(slice_at(t + AHEAD[p]), t + AHEAD[p], p)

    def run(t0, t1, work):
        last = t0 - GAP
        for t in range(t0, t1):
            advance(t)
            if work and work[0][0] <= t and t - last >= GAP:
                work.pop(0)[1]()
                last = t
        assert all(ready < t1 for ready, _ in work)
        for _, fn in work:
            fn()

    cp_x = pltpu.make_async_copy(x_hbm, x_v, sem_x)
    for t in range(NSEM):
        for p in (1, 0):
            if t < AHEAD[p]:
                start(stream(t), t, p)
        if t == 0:
            cp_x.start()

    cp_x.wait()
    x = x_v[...].astype(f32)
    xc = x - jnp.mean(x, axis=-1, keepdims=True)
    var = jnp.mean(xc * xc, axis=-1, keepdims=True)
    xn = jnp.broadcast_to(xc / jnp.sqrt(var + 1e-5), (ROWS, D)).astype(bf16)

    def project(w_v, col, width):
        w = w_v[:, :, pl.ds(col, width)].reshape(D, width)
        return jnp.dot(xn, w, preferred_element_type=f32)

    row = jax.lax.broadcasted_iota(jnp.int32, (ROWS, PAIR), 0)
    col = jax.lax.broadcasted_iota(jnp.int32, (ROWS, PAIR), 1)
    diag = row == (col >= DH).astype(jnp.int32)

    def query(j, i):
        c = j * PAIR + i * LANES
        q = project(wq_v, c if isinstance(j, int) else pl.multiple_of(c, LANES), LANES)
        q_s[j, :, pl.ds(i * LANES, LANES)] = jnp.where(
            diag[:, i * LANES:(i + 1) * LANES], q, 0.0).astype(bf16)

    run(0, head + kv_down, [(head - 1, lambda i=i: query(0, i)) for i in range(tiles)])

    scale = DH ** -0.5
    pieces = W // STEP

    def pair(j, last):
        slot = j % 2
        st = {}

        def scores(i):
            cols = pl.ds(i * STEP, STEP)
            s = jnp.dot(q_s[j], kbuf[slot, :, cols], preferred_element_type=f32) * scale
            s_s[:, cols] = s
            st["m"] = s if i == 0 else jnp.maximum(st["m"], s)
            if i == pieces - 1:
                st["m"] = jnp.max(st["m"], axis=-1, keepdims=True)
            if i < tiles and not last:
                query(j + 1, i)

        def values(i):
            cols = pl.ds(i * STEP, STEP)
            p = jnp.exp(s_s[:, cols] - st["m"])
            o = jax.lax.dot_general(p.astype(bf16), vbuf[slot, :, cols], _NT,
                                    preferred_element_type=f32)
            st["l"] = p if i == 0 else st["l"] + p
            st["o"] = o if i == 0 else st["o"] + o
            if i == pieces - 1:
                denom = jnp.sum(st["l"], axis=-1, keepdims=True)
                o_s[j] = jnp.where(diag, st["o"] / denom, 0.0).astype(bf16)

        done = 0
        for u in range(2 * kv_count):
            t = head + kv_down + u
            if last:
                advance(t + j * 2 * kv_count)
            else:
                advance(t, lambda t: kv_slice(j, t - head))
            while done <= u * pieces // kv_count:
                (scores if done < pieces else values)(done % pieces)
                done += 1

    def loop_body(j, carry):
        pair(j, False)
        return carry

    jax.lax.fori_loop(0, npairs - 1, loop_body, 0)
    pair(npairs - 1, True)

    st = {}

    def gate(n):
        st["g", n] = project(w1_v, n * STEP, STEP)

    def hidden(n):
        g = st["g", n]
        h = g * jax.nn.sigmoid(g) * project(w3_v, n * STEP, STEP)
        h_s[:, pl.ds(n * STEP, STEP)] = h.astype(bf16)

    def out_proj(blocks):
        for g, r in blocks:
            i = (g * wo_v.shape[1] + r) // LANES
            part = jnp.dot(o_s[i // tiles, :, pl.ds(i % tiles * LANES, LANES)],
                           wo_v[g, pl.ds(r, LANES), :], preferred_element_type=f32)
            st["attn"] = st["attn"] + part if "attn" in st else part
        if blocks[-1] == (wo_v.shape[0] - 1, wo_v.shape[1] - LANES):
            a_s[...] = jnp.sum(st["attn"], axis=0, keepdims=True)

    def down(r, n):
        part = jnp.dot(h_s[:, pl.ds(r, n)], w2_v[0, pl.ds(r, n), :],
                       preferred_element_type=f32)
        st["mlp"] = st["mlp"] + part if "mlp" in st else part

    t3 = tail + len(w1_sl)
    to = t3 + len(w3_sl)
    t2 = to + len(wo_sl)
    work = [(t3 - 1, lambda n=n: gate(n)) for n in range(F // STEP)]
    work += [(to - 1, lambda n=n: hidden(n)) for n in range(F // STEP)]
    work += [(to + _rows_ready(wo_sl, wo_v, r + LANES),
              lambda g=g, r=r: out_proj([(g, r), (g + 1, r)]))
             for r in range(0, wo_v.shape[1], LANES) for g in range(0, wo_v.shape[0], 2)]
    work += [(t2 + _rows_ready(w2_sl, w2_v, r + n), lambda r=r, n=n: down(r, n))
             for r, n in [(r, STEP) for r in range(0, F - STEP, STEP)]
             + [(r, LANES) for r in range(F - STEP, F, LANES)]]
    run(tail + kv_down, tail + len(tail_sl), work)

    mlp = st["mlp"][0:1]
    o_ref[...] = (x + a_s[...] * (mlp * jax.nn.sigmoid(mlp))).astype(o_ref.dtype)


@jax.jit
def pallas_recurrent_scan__sliding_block_cached__glu_gated_swiglu__decode_kernel(
    A_x: jax.Array,
    A_k_cache: jax.Array,
    A_v_cache: jax.Array,
    A_wq: jax.Array,
    A_wo: jax.Array,
    B_x: jax.Array,
    B_w1: jax.Array,
    B_w3: jax.Array,
    B_w2: jax.Array,
):
    del B_x
    B, Sq, D = A_x.shape
    _, H, Sk, Dh = A_k_cache.shape
    assert (B, Sq, H, Dh) == (1, 1, HQ, DH)
    W = min(4096, max(256, Sk // 4))
    kt = jnp.swapaxes(A_k_cache, 2, 3).reshape(H * Dh, Sk)
    vt = jnp.swapaxes(A_v_cache, 2, 3).reshape(H * Dh, Sk)
    weights = [w.reshape(shape[0], w.shape[0] // shape[0], w.shape[1])
               for w, shape in ((A_wq, WQ_SLICE), (A_wo, WO_SLICE), (B_w1, W13_SLICE),
                                (B_w3, W13_SLICE), (B_w2, W2_SLICE))]
    out = pl.pallas_call(
        _kernel,
        out_shape=jax.ShapeDtypeStruct((1, D), A_x.dtype),
        in_specs=[pl.BlockSpec(memory_space=pltpu.HBM)] * 8,
        out_specs=pl.BlockSpec(memory_space=pltpu.VMEM),
        scratch_shapes=[
            pltpu.VMEM((1, D), A_x.dtype),
            *[pltpu.VMEM(w.shape, w.dtype) for w in weights],
            pltpu.VMEM((2, PAIR, W), kt.dtype),
            pltpu.VMEM((2, PAIR, W), vt.dtype),
            pltpu.VMEM((H // 2, ROWS, PAIR), jnp.bfloat16),
            pltpu.VMEM((H // 2, ROWS, PAIR), jnp.bfloat16),
            pltpu.VMEM((ROWS, W), jnp.float32),
            pltpu.VMEM((ROWS, B_w1.shape[1]), jnp.bfloat16),
            pltpu.VMEM((1, D), jnp.float32),
        ],
        compiler_params=pltpu.CompilerParams(vmem_limit_bytes=64 * 1024 * 1024),
    )(A_x.reshape(1, D), kt, vt, *weights)
    return out.reshape(B, Sq, D)
```
